```python
import jax
import jax.numpy as jnp

def _softmax(x, axis=-1):
    return jax.nn.softmax(x, axis=axis)

def _gelu(x):
    return jax.nn.gelu(x, approximate=True)

def _silu(x):
    return jax.nn.silu(x)

def _sigmoid(x):
    return jax.nn.sigmoid(x)

def _layernorm(x, axis=-1, eps=1e-05):
    m = jnp.mean(x, axis=axis, keepdims=True)
    v = jnp.var(x, axis=axis, keepdims=True)
    return (x - m) / jnp.sqrt(v + eps)

def _scatter_add(tgt, idx, src, axis=0):
    return tgt.at[idx].add(src)

def _segment_sum(src, seg, n):
    return jax.ops.segment_sum(src, seg, n)

class _Rng:

    def __init__(self, key):
        self._k = key

    def _next(self):
        self._k, sub = jax.random.split(self._k)
        return sub

    def normal(self, shape):
        return jax.random.normal(self._next(), shape, dtype=jnp.bfloat16)

    def randint(self, lo, hi, shape):
        return jax.random.randint(self._next(), shape, lo, hi, dtype=jnp.int32)

    def uniform(self, shape, lo=0.0, hi=1.0):
        return jax.random.uniform(self._next(), shape, jnp.bfloat16, lo, hi)

    def permutation(self, n):
        return jax.random.permutation(self._next(), n)
kernel_name = 'adaLN_cond__grouped_kv_mqa__dense_activation_silu__prompt'

def _fwd_setup_inputs():
    _rng = _Rng(jax.random.key(int.from_bytes(__import__("os").urandom(4), "little")))
    _w = lambda a: (lambda t: t.astype(jnp.bfloat16) if jnp.issubdtype(t.dtype, jnp.floating) else t)(jnp.asarray(a))

    def _A_setup():
        B, S, D, H = (1, 2048, 640, 32)
        Dh = D // H
        return {'x': _w((lambda *s: _rng.normal(s) * 0.05)(B, S, D)), 'wq': _w((lambda *s: _rng.normal(s) * 0.05)(D, H * Dh)), 'wk': _w((lambda *s: _rng.normal(s) * 0.05)(D, Dh)), 'wv': _w((lambda *s: _rng.normal(s) * 0.05)(D, Dh)), 'wo': _w((lambda *s: _rng.normal(s) * 0.05)(H * Dh, D))}
    _A_in = _A_setup()

    def _B_setup():
        B, S, D, F = (1, 2048, 640, 1728)
        return {'x': _w((lambda *s: _rng.normal(s) * 0.05)(B, S, D)), 'w1': _w((lambda *s: _rng.normal(s) * 0.05)(D, F) * D ** (-0.5)), 'w2': _w((lambda *s: _rng.normal(s) * 0.05)(F, D) * F ** (-0.5))}
    _B_in = _B_setup()
    return {'A_x': _A_in['x'], 'A_wq': _A_in['wq'], 'A_wk': _A_in['wk'], 'A_wv': _A_in['wv'], 'A_wo': _A_in['wo'], 'B_x': _B_in['x'], 'B_w1': _B_in['w1'], 'B_w2': _B_in['w2'], 'c': _w((lambda *s: _rng.normal(s) * 0.05)(1, 640)), 'w_mod': _w((lambda *s: _rng.normal(s) * 0.05)(640, 6 * 640) * 640 ** (-0.5))}

def _fwd_reference(A_x, A_wq, A_wk, A_wv, A_wo, B_x, B_w1, B_w2, c, w_mod):

    def _A_ref(x, wq, wk, wv, wo):
        B, S, D = x.shape
        H = 32
        Dh = D // H
        q = (lambda x, *d: x.transpose(*d))((x @ wq).reshape(B, S, H, Dh), 0, 2, 1, 3)
        k = x @ wk
        v = x @ wv
        scores = jnp.einsum('bhqd,bkd->bhqk', q, k) * Dh ** (-0.5)
        p = _softmax(scores, axis=-1)
        o = jnp.einsum('bhqk,bkd->bhqd', p, v)
        return (lambda x, *d: x.transpose(*d))(o, 0, 2, 1, 3).reshape(B, S, H * Dh) @ wo

    def _B_ref(x, w1, w2):
        h = jnp.einsum('bsd,df->bsf', x, w1)
        h = _silu(h)
        out = jnp.einsum('bsf,fd->bsd', h, w2)
        return out
    x = A_x
    mod = (_silu(c) @ w_mod).reshape(c.shape[0], 6, 1, -1)
    sa, ca, ga, sb, cb, gb = (mod[:, 0].copy(), mod[:, 1].copy(), mod[:, 2].copy(), mod[:, 3].copy(), mod[:, 4].copy(), mod[:, 5].copy())
    h = _layernorm(x, axis=-1) * (1 + ca) + sa
    x = x + ga * _A_ref(h, A_wq, A_wk, A_wv, A_wo)
    h = _layernorm(x, axis=-1) * (1 + cb) + sb
    x = x + gb * _B_ref(h, B_w1, B_w2)
    return x

def setup_inputs():
    _inp = _fwd_setup_inputs()
    _gk = jax.random.fold_in(jax.random.key(int.from_bytes(__import__("os").urandom(4), "little")), 2 ** 31 - 1)
    _shapes = [[1, 2048, 640]]
    _dtypes = ['bfloat16']
    _gks = jax.random.split(_gk, len(_shapes))
    _gs = [jax.random.normal(k, s, dtype=jnp.dtype(d)) * 0.05 for k, s, d in zip(_gks, _shapes, _dtypes)]
    _inp['grad_out'] = _gs[0]
    return _inp

def reference(A_x, A_wq, A_wk, A_wv, A_wo, B_w1, B_w2, c, w_mod, B_x, grad_out):
    _const = dict(B_x=B_x)

    def _f(*_d):
        return _fwd_reference(**{'A_x': _d[0], 'A_wq': _d[1], 'A_wk': _d[2], 'A_wv': _d[3], 'A_wo': _d[4], 'B_w1': _d[5], 'B_w2': _d[6], 'c': _d[7], 'w_mod': _d[8], **_const})
    _out, _vjp = jax.vjp(_f, A_x, A_wq, A_wk, A_wv, A_wo, B_w1, B_w2, c, w_mod)
    _grads = _vjp(grad_out)
    _out0 = jnp.asarray(_out)
    return (_out0, *[jnp.asarray(_g) for _g in _grads])
```

```python
import math

import jax
import jax.numpy as jnp
from jax import lax
import jax.experimental.pallas as pl
import jax.experimental.pallas.tpu as pltpu

S = 2048
D = 640
H = 32
DH = 20
HP = 24
HD = H * HP
F = 1728
BQ = 256
NB = S // BQ
CK = 128
NCK = S // CK
EPS = 1e-5
SCALE = DH ** (-0.5)
LOG2E = math.log2(math.e)
LN2 = math.log(2.0)

FWD_SKEW = 5
FWD_HPI = 10
BWD_SKEW = 2
BWD_PPI = 4
HC = 192
RC = 64
SUB = 64
NQT = 6
SB1 = 64
QC = 80
UC = 160
FC2 = 288
FPER = 2
FP_ = 1792
NFB = FP_ // 128

XLU_COLS = (0, 2, 4)
XL = lambda j: j in XLU_COLS

f32 = jnp.float32
bf16 = jnp.bfloat16
NN = (((1,), (0,)), ((), ()))
NT = (((1,), (1,)), ((), ()))


def _dot(a, b, dims=NN):
    return lax.dot_general(a, b, dims, preferred_element_type=f32)


def _eye(n, m):
    r = lax.broadcasted_iota(jnp.int32, (n, m), 0)
    c = lax.broadcasted_iota(jnp.int32, (n, m), 1)
    return jnp.where(r == c, 1.0, 0.0).astype(bf16)


def _wide(cb):
    return jnp.concatenate([cb] * (BQ // 128), axis=1)


def _fold(v):
    out = v[:, 0:128]
    for t in range(1, BQ // 128):
        out = out + v[:, t * 128:(t + 1) * 128]
    return out


def _rsum(v):
    return jnp.sum(v.reshape(v.shape[0] // 8, 8, v.shape[1]), axis=0)


def _acc(a, v):
    return v if a is None else a + v


def _interleave(*streams):
    n = max(len(s) for s in streams)
    done = [0] * len(streams)
    for i in range(1, n + 1):
        for k, s in enumerate(streams):
            upto = (len(s) * i) // n
            while done[k] < upto:
                s[done[k]]()
                done[k] += 1


def _kernel(
    x_hbm, wq_hbm, wkT_ref, wvT_ref, wo_hbm, w1T_hbm, w2_hbm, c_ref, wmod_hbm, g_hbm,
    out_hbm, dx_hbm, dwq_hbm, dwkT_ref, dwvT_ref, dwo_hbm, dw1T_hbm, dw2_hbm, dc_ref, dwmod_hbm,
    *scratch_refs,
):
    (p_v, s0_v, s1_v, ds_v, knat_v, vnat_v, kTs_v, vTa_v, dkT_a, dvT_a, qT_v, oT_v, doT_v, dqT_v,
     oTn_v, dqb_v, linv_v, x_v, g_v, wmod_v, wqT_3, woT_3, w1_3, w2T_3,
     modb, xT_v, h1T_v, st1_v, h2T_v, dsl_v, dfT_v, daT_v, outT_v, dwo_a, dwq_a,
     dmod_a, dh1T_v, dx1T_v, ostage, dwmod_s, sT_v, duT_v, dw1_a, dw2_a, wq_v, wo_v, dwq_s,
     dwo_s, wkv_v, w1T_v, w2_v, dw1_s, dw2_s, m0_v, m1_v, wkvT_v, dwkv_a, dmod_r, in_sem,
     wm_sem, out_sem, wmo_sem, o_sem, x_sem) = scratch_refs

    def in_copy(i):
        src, dst = [(x_hbm, x_v), (wq_hbm, wq_v), (wo_hbm, wo_v),
                    (w1T_hbm, w1T_v.at[0:F, :]), (w2_hbm, w2_v.at[0:F, :]), (g_hbm, g_v)][i]
        return pltpu.make_async_copy(src, dst, in_sem.at[i])

    def x_copy(i):
        r0 = i * 2 * BQ if isinstance(i, int) else pl.multiple_of(i * 2 * BQ, 2 * BQ)
        return pltpu.make_async_copy(
            x_hbm.at[pl.ds(r0, 2 * BQ), :], x_v.at[pl.ds(r0, 2 * BQ), :], x_sem.at[i])

    def wmod_copy(i):
        return pltpu.make_async_copy(wmod_hbm.at[:, i * D:(i + 1) * D], wmod_v.at[i], wm_sem.at[i])

    def fin_copy(i):
        src, dst = [(dw1_s, dw1T_hbm), (dw2_s, dw2_hbm), (dwo_s, dwo_hbm), (dwq_s, dwq_hbm)][i]
        return pltpu.make_async_copy(src, dst, out_sem.at[i])

    def dwmod_copy(i):
        return pltpu.make_async_copy(dwmod_s.at[i], dwmod_hbm.at[:, i * D:(i + 1) * D], wmo_sem.at[i])

    def out_copy(dst_hbm, b, slot):
        return pltpu.make_async_copy(
            ostage.at[slot], dst_hbm.at[pl.ds(pl.multiple_of(b * BQ, BQ), BQ), :], o_sem.at[slot])

    wmod_copy(0).start()
    wmod_copy(1).start()
    x_copy(0).start()

    def transposed_chunk(src_v, b, j):
        xb = src_v[pl.ds(pl.multiple_of(b * BQ, BQ), BQ), j * 128:(j + 1) * 128]
        return _dot(_eye(128, 128), xb, NT)

    def transpose_rows(pairs, nblk, per):
        def one(src_v, dst3, use_xlu, i):
            eye128 = _eye(128, 128)
            r0 = i * 128 if isinstance(i, int) else pl.multiple_of(i * 128, 128)
            for j in range(src_v.shape[1] // 128):
                blk = src_v[pl.ds(r0, 128), j * 128:(j + 1) * 128]
                if use_xlu(j):
                    t = blk.astype(f32).T
                else:
                    t = _dot(eye128, blk, NT)
                dst3[i, j * 128:(j + 1) * 128, :] = t.astype(dst3.dtype)

        def body(i, carry):
            for k in range(per):
                for src_v, dst3, use_xlu in pairs:
                    one(src_v, dst3, use_xlu, i * per + k)
            return carry

        lax.fori_loop(0, nblk // per, body, 0)
        for i in range((nblk // per) * per, nblk):
            for src_v, dst3, use_xlu in pairs:
                one(src_v, dst3, use_xlu, i)

    def lhs3(ref3, rows):
        return jnp.concatenate([ref3[i, rows, :] for i in range(ref3.shape[0])], axis=1)

    def q_chunk(b, qs, r):
        nh = QC // DH
        if isinstance(r, int):
            rows = pl.ds(r * QC, QC)
            base = r * nh * HP
        else:
            rows = pl.ds(pl.multiple_of(r * QC, 16), QC)
            base = pl.multiple_of(r * nh * HP, 8)
        val = _dot(lhs3(wqT_3, rows), h1T_v[b]) * (SCALE * LOG2E)
        for j in range(nh):
            qT_v[qs, pl.ds(base + j * HP, DH), :] = val[j * DH:(j + 1) * DH, :]

    def set_mod(i):
        c_row = c_ref[...].astype(f32)
        sc_row = c_row / (1.0 + jnp.exp(-c_row))
        r = _dot(jnp.broadcast_to(sc_row, (8, D)), wmod_v[i])[0:1, :]
        r = r + jnp.where((i == 1) | (i == 4), 1.0, 0.0).astype(f32)
        modb[i] = jnp.broadcast_to(r, (128, D)).T

    def prologue():
        eye128 = _eye(128, 128)
        dkT_a[...] = jnp.zeros_like(dkT_a)
        dvT_a[...] = jnp.zeros_like(dvT_a)
        w1T_v[F:FP_, :] = jnp.zeros((FP_ - F, D), bf16)
        w2_v[F:FP_, :] = jnp.zeros((FP_ - F, D), bf16)
        sT_v[F:FP_, :] = jnp.zeros((FP_ - F, BQ), bf16)
        duT_v[F:FP_, :] = jnp.zeros((FP_ - F, BQ), bf16)

        def zero_body(i, carry):
            ds_v[pl.ds(pl.multiple_of(i * (S // 8), 16), S // 8), :] = jnp.zeros((S // 8, 2 * BQ), bf16)
            rows = pl.ds(pl.multiple_of(i * (HD // 8), 8), HD // 8)
            qT_v[:, rows, :] = jnp.zeros((2, HD // 8, BQ), f32)
            dmod_a[:, pl.ds(pl.multiple_of(i * (D // 8), 8), D // 8), :] = jnp.zeros((6, D // 8, 128), f32)
            return carry

        lax.fori_loop(0, 8, zero_body, 0)

        wkvT_v[...] = jnp.zeros_like(wkvT_v)
        wkvT_v[0:DH, :] = wkT_ref[...].astype(f32)
        wkvT_v[HP:HP + DH, :] = wvT_ref[...].astype(f32)
        for j in range(D // 128):
            wkv_v[j * 128:(j + 1) * 128, :] = _dot(
                eye128, wkvT_v[:, j * 128:(j + 1) * 128], NT).astype(bf16)

        c_row = c_ref[...].astype(f32)
        modb[6] = jnp.broadcast_to(c_row / (1.0 + jnp.exp(-c_row)), (128, D)).T

        wmod_copy(0).wait()
        wmod_copy(1).wait()
        x_copy(1).start()
        x_copy(2).start()
        set_mod(0)
        set_mod(1)


        def ln1_stage_t(b):
            s1 = None
            xs = []
            for j in range(D // 128):
                if XL(j):
                    xT = x_v[pl.ds(pl.multiple_of(b * BQ, BQ), BQ), j * 128:(j + 1) * 128].astype(f32).T
                else:
                    xT = transposed_chunk(x_v, b, j)
                xT_v[b, j * 128:(j + 1) * 128, :] = xT.astype(bf16)
                xs.append(xT)
                s1 = _acc(s1, _rsum(xT))
            return xs, s1

        def ln1_stage_n(b, xs, s1):
            mu = jnp.sum(s1, axis=0, keepdims=True) * (1.0 / D)
            s2 = None
            mc = mu
            for j in range(D // 128):
                for k in range(128 // SB1):
                    xc = xs[j][k * SB1:(k + 1) * SB1, :] - mc
                    s2 = _acc(s2, _rsum(xc * xc))
                    mc = mc + s2[0:1, :] * 0.0
            rstd = lax.rsqrt(jnp.sum(s2, axis=0, keepdims=True) * (1.0 / D) + EPS)
            st1_v[b, 0:1, :] = mu
            st1_v[b, 1:2, :] = rstd
            c1 = -mu * rstd
            rs = rstd
            hs = []
            for j in range(D // 128):
                for k in range(128 // SB1):
                    rows = slice(j * 128 + k * SB1, j * 128 + (k + 1) * SB1)
                    xh = xs[j][k * SB1:(k + 1) * SB1, :] * rs + c1
                    h = xh * _wide(modb[1, rows, :]) + _wide(modb[0, rows, :])
                    rs = rs + h[SB1 - 1:SB1, :] * 0.0
                    hs.append(h.astype(bf16))
                    h1T_v[b, rows, :] = hs[-1]
            return _dot(wkvT_v[...], jnp.concatenate(hs, axis=0))

        def ln1_stage_kv(b, kv):
            eye128 = _eye(128, 128)
            row = lax.broadcasted_iota(jnp.int32, (HP, BQ), 0)
            kT = kv[0:HP, :]
            vT = kv[HP:2 * HP, :]
            kTs_v[b] = kT * SCALE
            vTa_v[b] = jnp.where(row == DH, 1.0, vT)
            vT2 = jnp.where((row == DH) | (row == DH + 1), 1.0, vT)
            for t in range(BQ // 128):
                r0 = pl.multiple_of(b * BQ + t * 128, 128)
                knat_v[pl.ds(r0, 128), :] = _dot(
                    eye128, kT[:, t * 128:(t + 1) * 128], NT).astype(bf16)
                vnat_v[pl.ds(r0, 128), :] = _dot(
                    eye128, vT2[:, t * 128:(t + 1) * 128], NT).astype(bf16)

        def ln1_body(i, carry):
            x_copy(i).wait()

            @pl.when(i == 0)
            def _():
                x_copy(3).start()
                in_copy(1).start()

            @pl.when(i == 2)
            def _():
                for k in range(2, 6):
                    wmod_copy(k).start()
                for k in range(2, 6):
                    in_copy(k).start()

            ta = ln1_stage_t(2 * i)
            tb = ln1_stage_t(2 * i + 1)
            kva = ln1_stage_n(2 * i, *ta)
            kvb = ln1_stage_n(2 * i + 1, *tb)
            ln1_stage_kv(2 * i, kva)
            ln1_stage_kv(2 * i + 1, kvb)
            return carry

        lax.fori_loop(0, NB // 2, ln1_body, 0)

        in_copy(1).wait()
        transpose_rows([(wq_v, wqT_3, XL)], D // 128, D // 128)

        def q_body(r, carry):
            for k in range(4):
                q_chunk(0, 0, 4 * r + k)
            return carry

        lax.fori_loop(0, D // QC // 4, q_body, 0)

    def prologue2():
        def mod_body(i, carry):
            set_mod(2 * i)
            set_mod(2 * i + 1)
            return carry

        for i in range(2, 6):
            wmod_copy(i).wait()
        lax.fori_loop(1, 3, mod_body, 0)

        in_copy(2).wait()
        transpose_rows([(wo_v, woT_3, XL)], D // 128, D // 128)

        in_copy(3).wait()
        in_copy(4).wait()
        transpose_rows([(w1T_v, w1_3, XL), (w2_v, w2T_3, XL)], NFB, 2)
        in_copy(5).wait()

    sref = (s0_v, s1_v)
    mref = (m0_v, m1_v)

    def kvT_chunk(ref, c):
        per = BQ // CK
        return ref[c // per, :, (c % per) * CK:(c % per + 1) * CK]

    def q_rows(qs, h):
        return qT_v[qs, pl.ds(pl.multiple_of(h * HP, 8), HP), :]

    def a_step(q, par, c, m):
        s = _dot(knat_v[c * CK:(c + 1) * CK, :], q)
        sref[par][c * CK:(c + 1) * CK, :] = s
        mc = jnp.max(s.reshape(CK // 8, 8, BQ), axis=0)
        return mc if m is None else jnp.maximum(m, mc)

    def b_step(h, par, c, mB, acc):
        sb = sref[par][c * CK:(c + 1) * CK, :]
        p = jnp.exp2(sb - mB).astype(bf16)
        p_v[h, c * CK:(c + 1) * CK, :] = p
        d = _dot(kvT_chunk(vTa_v, c), p)
        return d if acc is None else acc + d

    def fwd_stage(qs, hA, parA, hB, hC, accC, filler=()):
        n, skew = NCK, FWD_SKEW
        filler = list(filler)
        if hA is not None:
            q = q_rows(qs, hA).astype(bf16)
        m = None
        accB = None
        if hC is not None:
            mC = mref[parA][0:1, :]
        for c in range(n):
            if filler:
                filler.pop(0)()
            if hA is not None:
                m = a_step(q, parA, c, m)
            if c < skew:
                if hC is not None:
                    accC = b_step(hC, parA, n - skew + c, mC, accC)
                    if c == skew - 1:
                        oT_v[pl.ds(pl.multiple_of(hC * HP, 8), HP), :] = accC
            elif hB is not None:
                if c == skew:
                    mB = mref[1 - parA][0:1, :]
                accB = b_step(hB, 1 - parA, c - skew, mB, accB)
        for fn in filler:
            fn()
        if hA is not None:
            mref[parA][...] = jnp.broadcast_to(jnp.max(m, axis=0, keepdims=True), (8, BQ))
        return accB

    def attn_fwd_main(qs):
        fwd_stage(qs, 0, 0, None, None, None)
        acc = fwd_stage(qs, 1, 1, 0, None, None)

        def body(i, acc):
            for j in range(FWD_HPI):
                h = FWD_HPI * i + 2 + j
                acc = fwd_stage(qs, h, j % 2, h - 1, h - 2, acc)
            return acc

        return lax.fori_loop(0, (H - 2) // FWD_HPI, body, acc)

    def attn_fwd_tail(acc, filler):
        acc = fwd_stage(None, None, 0, H - 1, H - 2, acc, filler)
        fwd_stage(None, None, 1, None, H - 1, acc)

    def p_pair(j, c):
        return jnp.concatenate(
            [p_v[2 * j, c * CK:(c + 1) * CK, :], p_v[2 * j + 1, c * CK:(c + 1) * CK, :]], axis=1)

    def pair_cols(w):
        return jnp.concatenate([w[0:HP, :], w[HP:2 * HP, :]], axis=1)

    def pair_rows(j):
        return pl.ds(pl.multiple_of(j * 2 * HP, 8), 2 * HP)

    def d_step(j, doTb, c):
        dp = _dot(vnat_v[c * CK:(c + 1) * CK, :], doTb)
        ds_v[c * CK:(c + 1) * CK, :] = (p_pair(j, c).astype(f32) * dp).astype(bf16)

    def e_step(j, qT, doT, c, acc):
        ds = ds_v[c * CK:(c + 1) * CK, :]
        dkT_a[:, c * CK:(c + 1) * CK] += _dot(qT, ds, NT)
        dvT_a[:, c * CK:(c + 1) * CK] += _dot(doT, p_pair(j, c), NT)
        d = _dot(kvT_chunk(kTs_v, c), ds)
        return d if acc is None else acc + d

    def bwd_stage(qs, jD, jC, accC, c_valid=None, filler=()):
        n, skew = NCK, BWD_SKEW
        filler = list(filler)
        if jD is not None:
            doT = pair_cols(doT_v[pair_rows(jD), :])
            qT = pair_cols(qT_v[qs, pair_rows(jD), :])
            doTb = doT.astype(bf16)
        doTC = pair_cols(doT_v[pair_rows(jC), :])
        qTC = pair_cols(qT_v[qs, pair_rows(jC), :])
        if c_valid is not None:
            vf = c_valid.astype(f32)
            doTC = doTC * vf
            qTC = qTC * vf
        acc = None
        for c in range(n):
            if filler:
                filler.pop(0)()
            if jD is not None:
                d_step(jD, doTb, c)
            if c < skew:
                accC = e_step(jC, qTC, doTC, n - skew + c, accC)
                if c == skew - 1:
                    dqT_v[pair_rows(jC), :] = jnp.concatenate(
                        [accC[:, 0:BQ], accC[:, BQ:2 * BQ]], axis=0)
            elif jD is not None:
                acc = e_step(jD, qT, doT, c - skew, acc)
        return acc

    def attn_bwd(qs, filler):
        def body(i, acc):
            for k in range(BWD_PPI):
                j = BWD_PPI * i + k
                acc = bwd_stage(qs, j, jnp.maximum(j - 1, 0), acc, (j > 0) if k == 0 else None)
            return acc

        acc = lax.fori_loop(0, H // 2 // BWD_PPI, body, jnp.zeros((HP, 2 * BQ), f32))
        for r in range(HD // HC - 1):
            dqb_chunk(r)
        bwd_stage(qs, None, H // 2 - 1, acc, None, filler)
        dqb_chunk(HD // HC - 1)

    def accumulate(ref, rows, val, first, stage=None):
        new = jnp.where(first, 0.0, ref[rows, :]) + val
        ref[rows, :] = new
        if stage is not None:
            stage[rows, :] = new.astype(bf16)

    def unpad_heads(v):
        n = v.shape[0] // HP
        return jnp.concatenate([v[j * HP:j * HP + DH, :] for j in range(n)], axis=0)

    def dqb_chunk(r):
        dqb_v[r * UC:(r + 1) * UC, :] = unpad_heads(dqT_v[r * HC:(r + 1) * HC, :]).astype(bf16)

    def dh1_chunk(b, rows):
        dh1T_v[b, rows, :] = _dot(wq_v[rows, :], dqb_v[...])

    def dwmod_slab(i):
        r = jnp.sum(dmod_a[i].T, axis=0, keepdims=True)
        dmod_r[i] = jnp.broadcast_to(r, (8, D))
        for k in range(D // RC):
            rows = slice(k * RC, (k + 1) * RC)
            scb = jnp.concatenate([modb[6, rows, :]] * (D // 128), axis=1)
            dwmod_s[i, rows, :] = (scb * r).astype(bf16)

    def dwmod_body(i, carry):
        dwmod_slab(i)
        return carry

    def ship_dense_grads():
        fin_copy(0).start()
        fin_copy(1).start()
        fin_copy(2).start()
        lax.fori_loop(2, 6, dwmod_body, 0)
        for i in range(2, 6):
            dwmod_copy(i).start()

    def epilogue():
        fin_copy(3).start()

        rowS = lax.broadcasted_iota(jnp.int32, (HP, BQ), 0)
        for b in range(NB):
            kTs_v[b] = jnp.where(rowS < DH, dkT_a[:, b * BQ:(b + 1) * BQ] * LN2, 0.0)
            vTa_v[b] = jnp.where(rowS < DH, dvT_a[:, b * BQ:(b + 1) * BQ], 0.0)
        dwkv_a[...] = jnp.zeros_like(dwkv_a)

        out_copy(out_hbm, NB - 2, 0).wait()
        out_copy(out_hbm, NB - 1, 1).wait()

        def fin_stage1(b):
            dkv = jnp.concatenate([kTs_v[b], vTa_v[b]], axis=0)
            dwkv_a[...] += _dot(dkv, h1T_v[b], NT)
            dkvb = dkv.astype(bf16)
            mu = st1_v[b, 0:1, :]
            rstd = st1_v[b, 1:2, :]
            s1 = None
            s2 = None
            dxh = []
            for r in range(D // RC):
                rows = slice(r * RC, (r + 1) * RC)
                dh1 = dh1T_v[b, rows, :] + _dot(wkv_v[rows, :], dkvb)
                xh = (xT_v[b, rows, :].astype(f32) - mu) * rstd
                dmod_a[0, rows, :] += _fold(dh1)
                dmod_a[1, rows, :] += _fold(dh1 * xh)
                dxh.append(dh1 * _wide(modb[1, rows, :]))
                s1 = _acc(s1, _rsum(dxh[-1]))
                s2 = _acc(s2, _rsum(dxh[-1] * xh))
            return dxh, s1, s2

        def fin_stage2(b, slot, dxh, s1, s2):
            mu = st1_v[b, 0:1, :]
            rstd = st1_v[b, 1:2, :]
            m1 = jnp.sum(s1, axis=0, keepdims=True) * (1.0 / D)
            m2 = jnp.sum(s2, axis=0, keepdims=True) * (1.0 / D)
            a2 = rstd * rstd * m2
            c2 = rstd * m1 - a2 * mu
            dxs = []
            for r in range(D // RC):
                rows = slice(r * RC, (r + 1) * RC)
                dxs.append(((dx1T_v[b, rows, :] - c2)
                            + (rstd * dxh[r] - xT_v[b, rows, :].astype(f32) * a2)).astype(bf16))
            dxT = jnp.concatenate(dxs, axis=0)
            eye128 = _eye(128, 128)
            for t in range(BQ // 128):
                ostage[slot, t * 128:(t + 1) * 128, :] = _dot(
                    eye128, dxT[:, t * 128:(t + 1) * 128], NT).astype(bf16)

        def fin_body(i, carry):
            s0 = (i % 2) * 2

            @pl.when(i >= 2)
            def _():
                out_copy(dx_hbm, 2 * i - 4, s0).wait()
                out_copy(dx_hbm, 2 * i - 3, s0 + 1).wait()

            ra = fin_stage1(2 * i)
            rb = fin_stage1(2 * i + 1)
            fin_stage2(2 * i, s0, *ra)
            fin_stage2(2 * i + 1, s0 + 1, *rb)
            out_copy(dx_hbm, 2 * i, s0).start()
            out_copy(dx_hbm, 2 * i + 1, s0 + 1).start()
            return carry

        lax.fori_loop(0, NB // 2, fin_body, 0)
        dwkT_ref[...] = dwkv_a[0:DH, :].astype(bf16)
        dwvT_ref[...] = dwkv_a[HP:HP + DH, :].astype(bf16)

        lax.fori_loop(0, 2, dwmod_body, 0)
        dwmod_copy(0).start()
        dwmod_copy(1).start()

        def dc_body(i, acc):
            return acc + _dot(dmod_r[i], wmod_v[i], NT)

        dsc = lax.fori_loop(0, 6, dc_body, jnp.zeros((8, D), f32))[0:1, :]
        c_row = c_ref[...].astype(f32)
        c_sig = 1.0 / (1.0 + jnp.exp(-c_row))
        dc_ref[...] = (dsc * (c_sig * (1.0 + c_row * (1.0 - c_sig)))).astype(bf16)

    def block_body(b, carry):
        slot = b % 2
        first = b == 0

        @pl.when(first)
        def _():
            prologue()

        @pl.when(b >= 2)
        def _():
            out_copy(out_hbm, b - 2, slot).wait()

        bnext = jnp.minimum(b + 1, NB - 1)
        chunks = lambda n: [slice(r * RC, (r + 1) * RC) for r in range(n // RC)]

        acc = attn_fwd_main(slot)

        @pl.when(first)
        def _():
            prologue2()

        NR = D // RC
        gT = [None] * NR

        def g_chunk(j):
            t = g_v[pl.ds(pl.multiple_of(b * BQ, BQ), BQ), j * 128:(j + 1) * 128].astype(f32).T
            for k in range(128 // RC):
                gT[j * (128 // RC) + k] = t[k * RC:(k + 1) * RC, :]

        qf = [lambda r=r: q_chunk(bnext, 1 - slot, r) for r in range(D // QC)]
        vf = [lambda j=j: g_chunk(j) for j in range(D // 128)]
        filler = []
        for k in range(NQT):
            filler += qf[k:k + 1] + vf[k:k + 1] + [lambda: None]
        attn_fwd_tail(acc, filler)

        def norm_chunk(r):
            o3 = oT_v[r * HC:(r + 1) * HC, :].reshape(HC // HP, HP, BQ)
            linv = 1.0 / o3[:, DH:DH + 1, :]
            linv_v[r] = jnp.broadcast_to(linv, (HC // HP, 8, BQ))
            on = (o3 * linv).reshape(HC, BQ)
            oT_v[r * HC:(r + 1) * HC, :] = on
            oTn_v[r * UC:(r + 1) * UC, :] = unpad_heads(on).astype(bf16)

        _interleave(qf[NQT:], [lambda r=r: norm_chunk(r) for r in range(HD // HC)])

        NT_ = BQ // 128
        lanes = [slice(t * 128, (t + 1) * 128) for t in range(NT_)]
        RH = 128
        hchunks = [slice(r * RH, (r + 1) * RH) for r in range(D // RH)]
        aT = [[None] * len(hchunks) for _ in range(NT_)]
        x1 = [[None] * len(hchunks) for _ in range(NT_)]
        mu2 = [None] * NT_
        rstd2 = [None] * NT_

        def proj_half(t):
            onb = oTn_v[:, lanes[t]]
            s1 = None
            for r, rows in enumerate(hchunks):
                a = _dot(lhs3(woT_3, rows), onb)
                aT[t][r] = a
                x1[t][r] = xT_v[b, rows, lanes[t]].astype(f32) + modb[2, rows, :] * a
                s1 = _acc(s1, _rsum(x1[t][r]))
            mu2[t] = jnp.sum(s1, axis=0, keepdims=True) * (1.0 / D)

        def ln2_half(t):
            s2 = None
            mu = mu2[t]
            for r in range(len(hchunks)):
                for k in range(RH // SUB):
                    xc = x1[t][r][k * SUB:(k + 1) * SUB, :] - mu
                    s2 = _acc(s2, _rsum(xc * xc))
                    mu = mu + s2[0:1, :] * 0.0
            rstd2[t] = lax.rsqrt(jnp.sum(s2, axis=0, keepdims=True) * (1.0 / D) + EPS)
            c2 = -mu2[t] * rstd2[t]
            rs = rstd2[t]
            for r in range(len(hchunks)):
                for k in range(RH // SUB):
                    srows = slice(r * RH + k * SUB, r * RH + (k + 1) * SUB)
                    xh = x1[t][r][k * SUB:(k + 1) * SUB, :] * rs + c2
                    h2 = xh * modb[4, srows, :] + modb[3, srows, :]
                    h2T_v[srows, lanes[t]] = h2.astype(bf16)
                    rs = rs + h2[SUB - 1:SUB, :] * 0.0

        def up_half(t):
            h2b = h2T_v[:, lanes[t]]
            for r in range(F // FC2):
                rows = slice(r * FC2, (r + 1) * FC2)
                u = _dot(w1T_v[rows, :], h2b)
                sg = 0.5 * jnp.tanh(0.5 * u) + 0.5
                sT_v[rows, lanes[t]] = (u * sg).astype(bf16)
                dsl_v[rows, lanes[t]] = sg * (1.0 + u * (1.0 - sg))

        proj_half(0)
        proj_half(1)
        ln2_half(0)
        up_half(0)
        ln2_half(1)
        up_half(1)

        def cat(vals, r):
            k, o = divmod(r * RC, RH)
            return jnp.concatenate([vals[t][k][o:o + RC, :] for t in range(NT_)], axis=1)

        sb_ = sT_v[...]
        for r, rows in enumerate(chunks(D)):
            fT = _dot(lhs3(w2T_3, rows), sb_)
            gbw = _wide(modb[5, rows, :])
            outT_v[rows, :] = (cat(x1, r) + gbw * fT).astype(bf16)
            dmod_a[5, rows, :] += _fold(gT[r] * fT)
            dfT_v[rows, :] = (gT[r] * gbw).astype(bf16)

        def mlp_bwd_body(i, carry):
            dfb = dfT_v[...]
            h2b_ = h2T_v[...]
            for k in range(FPER):
                rows = pl.ds(pl.multiple_of((i * FPER + k) * FC2, 16), FC2)
                dsT = _dot(w2_v[rows, :], dfb)
                du = (dsT * dsl_v[rows, :]).astype(bf16)
                duT_v[rows, :] = du
                accumulate(dw2_a, rows, _dot(sT_v[rows, :], dfb, NT), first, dw2_s)
                accumulate(dw1_a, rows, _dot(du, h2b_, NT), first, dw1_s)
            return carry

        lax.fori_loop(0, F // FC2 // FPER, mlp_bwd_body, 0)
        for t in range(BQ // 128):
            ostage[slot, t * 128:(t + 1) * 128, :] = outT_v[:, t * 128:(t + 1) * 128].astype(f32).T.astype(bf16)
        out_copy(out_hbm, b, slot).start()
        dxh = [[None] * len(hchunks) for _ in range(NT_)]
        msum = [None] * NT_

        def down_chunk(t, r):
            rows = hchunks[r]
            dh2 = _dot(lhs3(w1_3, rows), duT_v[:, lanes[t]])
            xh = (x1[t][r] - mu2[t]) * rstd2[t]
            dmod_a[3, rows, :] += dh2
            dmod_a[4, rows, :] += dh2 * xh
            dx = dh2 * modb[4, rows, :]
            s1, s2 = msum[t] if msum[t] is not None else (None, None)
            msum[t] = (_acc(s1, _rsum(dx)), _acc(s2, _rsum(dx * xh)))
            g = jnp.concatenate([gT[2 * r][:, lanes[t]], gT[2 * r + 1][:, lanes[t]]], axis=0)
            dxh[t][r] = g + rstd2[t] * dx

        lnb = [None] * NT_

        def ln2_bwd_chunk(t, r):
            rows = hchunks[r]
            if lnb[t] is None:
                m1 = jnp.sum(msum[t][0], axis=0, keepdims=True) * (1.0 / D)
                m2 = jnp.sum(msum[t][1], axis=0, keepdims=True) * (1.0 / D)
                a2 = rstd2[t] * rstd2[t] * m2
                lnb[t] = (a2, rstd2[t] * m1 - a2 * mu2[t])
            for k in range(RH // SUB):
                a2, c2 = lnb[t]
                sub = slice(k * SUB, (k + 1) * SUB)
                srows = slice(r * RH + k * SUB, r * RH + (k + 1) * SUB)
                dx1 = dxh[t][r][sub, :] - (x1[t][r][sub, :] * a2 + c2)
                dx1T_v[b, srows, lanes[t]] = dx1
                dmod_a[2, srows, :] += dx1 * aT[t][r][sub, :]
                daT_v[srows, lanes[t]] = (dx1 * modb[2, srows, :]).astype(bf16)
                lnb[t] = (a2 + dx1[SUB - 1:SUB, :] * 0.0, c2)

        zrow = jnp.zeros((HP - DH, 128), f32)

        def do_half(t):
            dab = daT_v[:, lanes[t]]
            for r in range(HD // HC):
                rows = slice(r * HC, (r + 1) * HC)
                dou = _dot(wo_v[r * UC:(r + 1) * UC, :], dab)
                parts = []
                for j in range(HC // HP):
                    parts += [dou[j * DH:(j + 1) * DH, :], zrow]
                do3 = jnp.concatenate(parts, axis=0).reshape(HC // HP, HP, 128)
                o3 = oT_v[rows, lanes[t]].reshape(HC // HP, HP, 128)
                linv = linv_v[r][:, 0:1, lanes[t]]
                do3 = do3 * linv
                delta = jnp.sum(do3 * o3, axis=1, keepdims=True)
                d_hi = delta.astype(bf16).astype(f32)
                d_lo = delta - d_hi
                row = lax.broadcasted_iota(jnp.int32, (HC // HP, HP, 128), 1)
                do3 = jnp.where(row == DH, -d_hi, jnp.where(row == DH + 1, -d_lo, do3))
                doT_v[rows, lanes[t]] = do3.reshape(HC, 128)

        nh_ = len(hchunks)
        for r in range(nh_):
            down_chunk(0, r)
        for r in range(nh_):
            down_chunk(1, r)
            ln2_bwd_chunk(0, r)
        do_half(0)
        for r in range(nh_):
            ln2_bwd_chunk(1, r)
        do_half(1)
        dab = daT_v[...]
        for r in range(HD // HC):
            urows = slice(r * UC, (r + 1) * UC)
            accumulate(dwo_a, urows, _dot(oTn_v[urows, :], dab, NT), first, dwo_s)

        @pl.when(b == NB - 1)
        def _():
            ship_dense_grads()

        def dwq_part(rows, c0, c1):
            new = (jnp.where(first, 0.0, dwq_a[rows, c0:c1])
                   + _dot(h1T_v[b, rows, :], dqb_v[c0:c1, :], NT))
            dwq_a[rows, c0:c1] = new
            dwq_s[rows, c0:c1] = new.astype(bf16)

        attn_bwd(slot, [lambda rows=rows: dwq_part(rows, 0, 384) for rows in hchunks])
        for rows in hchunks:
            dwq_part(rows, 384, D)
        for rows in chunks(D):
            dh1_chunk(b, rows)
        return carry

    lax.fori_loop(0, NB, block_body, 0)
    epilogue()

    for k in range(4):
        out_copy(dx_hbm, NB - 4 + k, k).wait()
    for i in range(4):
        fin_copy(i).wait()
    for i in range(6):
        dwmod_copy(i).wait()


@jax.jit
def pallas_adaLN_cond__grouped_kv_mqa__dense_activation_silu__prompt_kernel(
    A_x: jax.Array,
    A_wq: jax.Array,
    A_wk: jax.Array,
    A_wv: jax.Array,
    A_wo: jax.Array,
    B_x: jax.Array,
    B_w1: jax.Array,
    B_w2: jax.Array,
    c: jax.Array,
    w_mod: jax.Array,
    grad_out: jax.Array,
):
    x = A_x.reshape(S, D)
    g = grad_out.reshape(S, D)

    any_spec = pl.BlockSpec(memory_space=pl.ANY)
    vmem_spec = pl.BlockSpec(memory_space=pltpu.VMEM)
    V = pltpu.VMEM

    out_shape = (
        jax.ShapeDtypeStruct((S, D), bf16),
        jax.ShapeDtypeStruct((S, D), bf16),
        jax.ShapeDtypeStruct((D, D), bf16),
        jax.ShapeDtypeStruct((DH, D), bf16),
        jax.ShapeDtypeStruct((DH, D), bf16),
        jax.ShapeDtypeStruct((D, D), bf16),
        jax.ShapeDtypeStruct((F, D), bf16),
        jax.ShapeDtypeStruct((F, D), bf16),
        jax.ShapeDtypeStruct((1, D), bf16),
        jax.ShapeDtypeStruct((D, 6 * D), bf16),
    )
    scratch = [
        V((H, S, BQ), bf16),
        V((S, BQ), f32),
        V((S, BQ), f32),
        V((S, 2 * BQ), bf16),
        V((S, HP), bf16),
        V((S, HP), bf16),
        V((NB, HP, BQ), f32),
        V((NB, HP, BQ), f32),
        V((HP, S), f32),
        V((HP, S), f32),
        V((2, HD, BQ), f32),
        V((HD, BQ), f32),
        V((HD, BQ), f32),
        V((HD, BQ), f32),
        V((D, BQ), bf16),
        V((D, BQ), bf16),
        V((HD // HC, HC // HP, 8, BQ), f32),
        V((S, D), bf16),
        V((S, D), bf16),
        V((6, D, D), bf16),
        V((D // 128, D, 128), bf16),
        V((D // 128, D, 128), bf16),
        V((NFB, D, 128), bf16),
        V((NFB, D, 128), bf16),
        V((7, D, 128), f32),
        V((NB, D, BQ), bf16),
        V((NB, D, BQ), bf16),
        V((NB, 8, BQ), f32),
        V((D, BQ), bf16),
        V((F, BQ), f32),
        V((D, BQ), bf16),
        V((D, BQ), bf16),
        V((D, BQ), bf16),
        V((D, D), f32),
        V((D, D), f32),
        V((6, D, 128), f32),
        V((NB, D, BQ), f32),
        V((NB, D, BQ), f32),
        V((4, BQ, D), bf16),
        V((6, D, D), bf16),
        V((FP_, BQ), bf16),
        V((FP_, BQ), bf16),
        V((F, D), f32),
        V((F, D), f32),
        V((D, D), bf16),
        V((D, D), bf16),
        V((D, D), bf16),
        V((D, D), bf16),
        V((D, 2 * HP), bf16),
        V((FP_, D), bf16),
        V((FP_, D), bf16),
        V((F, D), bf16),
        V((F, D), bf16),
        V((8, BQ), f32),
        V((8, BQ), f32),
        V((2 * HP, D), f32),
        V((2 * HP, D), f32),
        V((6, 8, D), f32),
        pltpu.SemaphoreType.DMA((6,)), pltpu.SemaphoreType.DMA((6,)), pltpu.SemaphoreType.DMA((4,)),
        pltpu.SemaphoreType.DMA((6,)), pltpu.SemaphoreType.DMA((4,)),
        pltpu.SemaphoreType.DMA((NB // 2,)),
    ]
    outs = pl.pallas_call(
        _kernel,
        out_shape=out_shape,
        in_specs=[any_spec, any_spec, vmem_spec, vmem_spec, any_spec, any_spec, any_spec,
                  vmem_spec, any_spec, any_spec],
        out_specs=(any_spec, any_spec, any_spec, vmem_spec, vmem_spec, any_spec, any_spec,
                   any_spec, vmem_spec, any_spec),
        scratch_shapes=scratch,
        compiler_params=pltpu.CompilerParams(vmem_limit_bytes=127 * 1024 * 1024),
    )(x, A_wq, A_wk.T, A_wv.T, A_wo, B_w1.T, B_w2, c, w_mod, g)
    out, dx, dwq, dwkT, dwvT, dwo, dw1T, dw2, dc, dwmod = outs
    return (out.reshape(1, S, D), dx.reshape(1, S, D), dwq, dwkT.T, dwvT.T, dwo, dw1T.T, dw2, dc,
            dwmod)
```
